```python
import jax
import jax.numpy as jnp

def _softmax(x, axis=-1):
    return jax.nn.softmax(x, axis=axis)

def _gelu(x):
    return jax.nn.gelu(x, approximate=True)

def _silu(x):
    return jax.nn.silu(x)

def _sigmoid(x):
    return jax.nn.sigmoid(x)

def _layernorm(x, axis=-1, eps=1e-05):
    m = jnp.mean(x, axis=axis, keepdims=True)
    v = jnp.var(x, axis=axis, keepdims=True)
    return (x - m) / jnp.sqrt(v + eps)

def _scatter_add(tgt, idx, src, axis=0):
    return tgt.at[idx].add(src)

def _segment_sum(src, seg, n):
    return jax.ops.segment_sum(src, seg, n)

class _Rng:

    def __init__(self, key):
        self._k = key

    def _next(self):
        self._k, sub = jax.random.split(self._k)
        return sub

    def normal(self, shape):
        return jax.random.normal(self._next(), shape, dtype=jnp.bfloat16)

    def randint(self, lo, hi, shape):
        return jax.random.randint(self._next(), shape, lo, hi, dtype=jnp.int32)

    def uniform(self, shape, lo=0.0, hi=1.0):
        return jax.random.uniform(self._next(), shape, jnp.bfloat16, lo, hi)

    def permutation(self, n):
        return jax.random.permutation(self._next(), n)
kernel_name = 'sequential_preLN__ssm_conv_s4__mixer_gmlp__prompt'

def _fwd_setup_inputs():
    _rng = _Rng(jax.random.key(int.from_bytes(__import__("os").urandom(4), "little")))
    _w = lambda a: (lambda t: t.astype(jnp.bfloat16) if jnp.issubdtype(t.dtype, jnp.floating) else t)(jnp.asarray(a))

    def _A_setup():
        B, L, D, N = (1, 2048, 576, 128)
        A_re = -jnp.exp((lambda *s: _rng.normal(s) * 0.05)(D, N))
        A_im = jnp.pi * (lambda *s: _rng.normal(s) * 0.05)(D, N)
        B_re = (lambda *s: _rng.normal(s) * 0.05)(D, N)
        B_im = (lambda *s: _rng.normal(s) * 0.05)(D, N)
        C_re = (lambda *s: _rng.normal(s) * 0.05)(D, N)
        C_im = (lambda *s: _rng.normal(s) * 0.05)(D, N)
        log_dt = (lambda *s: _rng.normal(s) * 0.05)(D) * 0.5 - 4.0
        Dskip = (lambda *s: _rng.normal(s) * 0.05)(D)
        return {'u': _w((lambda *s: _rng.normal(s) * 0.05)(B, L, D)), 'A_re': _w(A_re), 'A_im': _w(A_im), 'B_re': _w(B_re), 'B_im': _w(B_im), 'C_re': _w(C_re), 'C_im': _w(C_im), 'log_dt': _w(log_dt), 'Dskip': _w(Dskip)}
    _A_in = _A_setup()

    def _B_setup():
        B, S, D, F = (1, 2048, 576, 4608)
        Fh = F // 2
        return {'x': _w((lambda *s: _rng.normal(s) * 0.05)(B, S, D)), 'w_in': _w((lambda *s: _rng.normal(s) * 0.05)(D, 2 * Fh)), 'w_sp': _w(0.01 * (lambda *s: _rng.normal(s) * 0.05)(S, S)), 'b_sp': _w(1.0 + 0.01 * (lambda *s: _rng.normal(s) * 0.05)(S)), 'w_out': _w((lambda *s: _rng.normal(s) * 0.05)(Fh, D))}
    _B_in = _B_setup()
    return {'A_u': _A_in['u'], 'A_A_re': _A_in['A_re'], 'A_A_im': _A_in['A_im'], 'A_B_re': _A_in['B_re'], 'A_B_im': _A_in['B_im'], 'A_C_re': _A_in['C_re'], 'A_C_im': _A_in['C_im'], 'A_log_dt': _A_in['log_dt'], 'A_Dskip': _A_in['Dskip'], 'B_x': _B_in['x'], 'B_w_in': _B_in['w_in'], 'B_w_sp': _B_in['w_sp'], 'B_b_sp': _B_in['b_sp'], 'B_w_out': _B_in['w_out']}

def _fwd_reference(A_u, A_A_re, A_A_im, A_B_re, A_B_im, A_C_re, A_C_im, A_log_dt, A_Dskip, B_x, B_w_in, B_w_sp, B_b_sp, B_w_out):

    def _A_ref(u, A_re, A_im, B_re, B_im, C_re, C_im, log_dt, Dskip):
        Bsz, L, D = u.shape
        dt = jnp.exp(log_dt)[:, None]
        A = A_re + 1j * A_im
        Bc = B_re + 1j * B_im
        Cc = C_re + 1j * C_im
        logdA = dt * A
        dB = dt * Bc
        l = (lambda x, dt: x.astype(dt))(jnp.arange(L), A_re.dtype)
        P = jnp.exp(logdA[:, :, None] * l[None, None, :])
        K = jnp.einsum('dn,dnl,dn->dl', Cc, P, dB).real
        L2 = 2 * L
        Kp = jnp.pad(K, ((0, 0), (0, L)))
        up = (lambda x, *d: x.transpose(*d))(u, 0, 2, 1)
        up = jnp.pad(up, ((0, 0), (0, 0), (0, L)))
        Kf = (lambda x, axes=(-2, -1): jnp.fft.rfft2(x.astype(jnp.float32), axes=axes))(Kp[:, None, :], axes=(-2, -1))
        Uf = (lambda x, axes=(-2, -1): jnp.fft.rfft2(x.astype(jnp.float32), axes=axes))(up[:, :, None, :], axes=(-2, -1))
        Yf = Uf * Kf[None, :, :, :]
        y = (lambda x, s, axes=(-2, -1): jnp.fft.irfft2(x, s=s, axes=axes).astype(jnp.bfloat16))(Yf, (1, L2), axes=(-2, -1))[:, :, 0, :L]
        y = (lambda x, *d: x.transpose(*d))(y, 0, 2, 1) + u * Dskip[None, None, :]
        return y

    def _B_ref(x, w_in, w_sp, b_sp, w_out):
        B, S, D = x.shape
        F = w_in.shape[-1]
        Fh = F // 2
        z = _gelu(jnp.einsum('bsd,df->bsf', x, w_in))
        z1 = z[..., :Fh].copy()
        z2 = _layernorm(z[..., Fh:], axis=-1)
        g = jnp.einsum('ts,bsf->btf', w_sp, z2) + b_sp[None, :, None]
        return jnp.einsum('bsf,fd->bsd', z1 * g, w_out)
    x = A_u
    h = x + _A_ref(_layernorm(x, axis=-1), A_A_re, A_A_im, A_B_re, A_B_im, A_C_re, A_C_im, A_log_dt, A_Dskip)
    h2 = h + _B_ref(_layernorm(h, axis=-1), B_w_in, B_w_sp, B_b_sp, B_w_out)
    return h2

def setup_inputs():
    _inp = _fwd_setup_inputs()
    _gk = jax.random.fold_in(jax.random.key(int.from_bytes(__import__("os").urandom(4), "little")), 2 ** 31 - 1)
    _shapes = [[1, 2048, 576]]
    _dtypes = ['bfloat16']
    _gks = jax.random.split(_gk, len(_shapes))
    _gs = [jax.random.normal(k, s, dtype=jnp.dtype(d)) * 0.05 for k, s, d in zip(_gks, _shapes, _dtypes)]
    _inp['grad_out'] = _gs[0]
    return _inp

def reference(A_u, A_A_re, A_A_im, A_B_re, A_B_im, A_C_re, A_C_im, A_log_dt, A_Dskip, B_w_in, B_w_sp, B_b_sp, B_w_out, B_x, grad_out):
    _const = dict(B_x=B_x)

    def _f(*_d):
        return _fwd_reference(**{'A_u': _d[0], 'A_A_re': _d[1], 'A_A_im': _d[2], 'A_B_re': _d[3], 'A_B_im': _d[4], 'A_C_re': _d[5], 'A_C_im': _d[6], 'A_log_dt': _d[7], 'A_Dskip': _d[8], 'B_w_in': _d[9], 'B_w_sp': _d[10], 'B_b_sp': _d[11], 'B_w_out': _d[12], **_const})
    _out, _vjp = jax.vjp(_f, A_u, A_A_re, A_A_im, A_B_re, A_B_im, A_C_re, A_C_im, A_log_dt, A_Dskip, B_w_in, B_w_sp, B_b_sp, B_w_out)
    _grads = _vjp(grad_out)
    _out0 = jnp.asarray(_out)
    return (_out0, *[jnp.asarray(_g) for _g in _grads])
```

```python
import functools
import jax
import jax.numpy as jnp
from jax import lax
import jax.experimental.pallas as pl
import jax.experimental.pallas.tpu as pltpu

L, D, N, FH = 2048, 576, 128, 2304
PAD = 80
RB = 64
TM = 256
NQ = 648
LANES = [(0, 128), (128, 128), (256, 128), (384, 128), (512, 64)]
REG = [(0, 0, 1, 16), (256, 256, 2, 8), (384, 512, 4, 8), (512, 1024, 8, 8)]
CREG = [
    (0, 0, 8, 32, [(r, 0) for r in range(8)]),
    (256, 256, 8, 32, [(8, 0), (2, 0), (9, 0), (6, 0)]),
    (384, 512, 8, 64, [(10, 0), (9, 0)]),
    (512, 1024, 16, 65, [(12, 0), (11, 8)]),
]
f32, bf16 = jnp.float32, jnp.bfloat16
_C0 = 0.7978845608028654


def _ln(x):
    m = jnp.mean(x, axis=-1, keepdims=True)
    c = x - m
    v = jnp.mean(c * c, axis=-1, keepdims=True)
    r = lax.rsqrt(v + 1e-5)
    return c * r, r


def _ln_bwd(xh, r, dy):
    a = jnp.mean(dy, axis=-1, keepdims=True)
    b = jnp.mean(dy * xh, axis=-1, keepdims=True)
    return r * (dy - a - xh * b)


def _gelu(x):
    return 0.5 * x * (1.0 + jnp.tanh(_C0 * (x + 0.044715 * x * x * x)))


def _gelu_grad(x):
    t = jnp.tanh(_C0 * (x + 0.044715 * x * x * x))
    return 0.5 * (1.0 + t) + 0.5 * x * (1.0 - t * t) * _C0 * (1.0 + 0.134145 * x * x)


def _dot(a, b):
    return jnp.dot(a, b, preferred_element_type=f32)


def _dot_nt(a, b):
    return lax.dot_general(a, b, (((1,), (1,)), ((), ())), preferred_element_type=f32)


def _kernel(x_ref, are_ref, aim_ref, bre_ref, bim_ref, cre_ref, cim_ref, ldt_ref, dsk_ref,
            win_ref, wsp_ref, wspt_ref, bsp_ref, wout_ref, go_ref,
            out_ref, dx_ref, dare_ref, daim_ref, dbre_ref, dbim_ref, dcre_ref, dcim_ref,
            dldt_ref, ddsk_ref, dwin_ref, dwsp_ref, dbsp_ref, dwoutt_ref,
            u_s, h_s, x2_s, kt_s):
    nblk = L // TM

    def rows(i):
        return pl.ds(pl.multiple_of(i * TM, TM), TM)

    def ln1(i, c):
        xh, _ = _ln(x_ref[rows(i), :].astype(f32))
        u_s[rows(i), :] = xh.astype(bf16)
        return c
    lax.fori_loop(0, nblk, ln1, 0)

    kt_full = kt_s
    dh_s = x2_s
    def ssm(fwd_pass, sh_s, up_s, lo_s, dk_s, y_s):
        kt_s = kt_full
        def ssm_params(c0, w):
            sl = slice(c0, c0 + w)
            dt = jnp.exp(ldt_ref[:, sl].astype(f32)).astype(bf16).astype(f32)
            A_r, A_i = are_ref[:, sl].astype(f32), aim_ref[:, sl].astype(f32)
            B_r, B_i = bre_ref[:, sl].astype(f32), bim_ref[:, sl].astype(f32)
            C_r, C_i = cre_ref[:, sl].astype(f32), cim_ref[:, sl].astype(f32)
            ar, ai = dt * A_r, dt * A_i
            dbr, dbi = dt * B_r, dt * B_i
            wr, wi = C_r * dbr - C_i * dbi, C_r * dbi + C_i * dbr
            return dt, A_r, A_i, B_r, B_i, C_r, C_i, ar, ai, dbr, dbi, wr, wi

        def cexp(ar, ai, l):
            e = jnp.exp(ar * l)
            return e * jnp.cos(ai * l), e * jnp.sin(ai * l)

        def build_lo(ar, ai, w):
            for g, (_, _, s, _) in enumerate(REG):
                for b in range(16):
                    er, ei = cexp(ar, ai, float(s * b))
                    lo_s[g, b, 0, :, :w] = er
                    lo_s[g, b, 1, :, :w] = ei

        def build_sh(src, c0, w, sign):
            o = 8 + PAD
            up_s[...] = jnp.zeros(up_s.shape, f32)
            up_s[o:o + L, :w] = src[:, c0:c0 + w].astype(f32)
            R = L + 2 * PAD

            def sh(k):
                return up_s[8 - sign * k:8 - sign * k + R, :w]
            for r in range(8):
                sh_s[r, :, :w] = sh(r)
            s3 = sh(-1) + sh(0) + sh(1)
            sh_s[8, :, :w] = s3
            sh_s[9, :, :w] = sh(3) + sh(4) + sh(5)
            s5 = s3 + sh(-2) + sh(2)
            sh_s[10, :, :w] = s5
            s7 = s5 + sh(-3) + sh(3)
            sh_s[11, :, :w] = s7
            sh_s[12, :, :w] = s7 + sh(-4) + sh(4)

        def conv(w, sign):
            def blk(i, c):
                t0 = i * RB
                span = (t0 + RB) if sign > 0 else (L - t0)
                acc = jnp.zeros((RB, w), f32)
                for (rb, lb, ps, npp, terms) in CREG:
                    ni = len(terms)

                    def body(p, acc, rb=rb, lb=lb, ps=ps, terms=terms, ni=ni):
                        for j, (a, eo) in enumerate(terms):
                            k = kt_s[pl.ds(rb + ni * p + j, 1), :w]
                            st = PAD + t0 - sign * (lb + ps * p + eo)
                            acc = acc + k * sh_s[a, pl.ds(pl.multiple_of(st, 8), RB), :w]
                        return acc
                    hi = jnp.clip((span + 8 - lb) // ps + 1, 0, npp)
                    acc = lax.fori_loop(0, hi, body, acc)
                @pl.when(span > 1016)
                def _():
                    k = kt_s[pl.ds(641, 1), :w]
                    st = PAD + t0 - sign * 1016
                    e = sh_s[4, pl.ds(pl.multiple_of(st, 8), RB), :w] + sh_s[5, pl.ds(pl.multiple_of(st, 8), RB), :w]
                    y_s[pl.ds(pl.multiple_of(t0, 8), RB), :w] = acc + k * e

                @pl.when(span <= 1016)
                def _():
                    y_s[pl.ds(pl.multiple_of(t0, 8), RB), :w] = acc
                return c
            lax.fori_loop(0, L // RB, blk, 0)

        if fwd_pass:
            for (c0, w) in LANES:
                dt, A_r, A_i, B_r, B_i, C_r, C_i, ar, ai, dbr, dbi, wr, wi = ssm_params(c0, w)
                build_lo(ar, ai, w)
                for g, (rb, lb, s, nh) in enumerate(REG):
                    def kbody(a, c, g=g, rb=rb, lb=lb, s=s):
                        er, ei = cexp(ar, ai, (lb + 16 * s * a).astype(f32))
                        hr, hi = wr * er - wi * ei, wr * ei + wi * er
                        for half in range(2):
                            rws = [jnp.sum(hr * lo_s[g, b, 0, :, :w] - hi * lo_s[g, b, 1, :, :w], axis=0, keepdims=True)
                                   for b in range(8 * half, 8 * half + 8)]
                            kt_s[pl.ds(pl.multiple_of(rb + 16 * a + 8 * half, 8), 8), c0:c0 + w] = jnp.concatenate(rws, axis=0)
                        return c
                    lax.fori_loop(0, nh, kbody, 0)
                er, ei = cexp(ar, ai, 2048.0)
                k2048 = jnp.sum(wr * er - wi * ei, axis=0, keepdims=True)
                k1024 = kt_s[512:513, c0:c0 + w]
                kt_s[640:648, c0:c0 + w] = jnp.concatenate(
                    [k2048, -k1024] + [jnp.zeros_like(k2048)] * 6, axis=0)
                kt_s[255:256, c0:c0 + w] = kt_s[255:256, c0:c0 + w] - kt_s[256:257, c0:c0 + w]
                kt_s[383:384, c0:c0 + w] = kt_s[383:384, c0:c0 + w] - kt_s[384:385, c0:c0 + w]

            for (c0, w) in LANES:
                build_sh(u_s, c0, w, 1)
                kt_s = kt_full.at[:, c0:c0 + w] if False else kt_full
                kt_s = dk_s
                dk_s[:, :w] = kt_full[:, c0:c0 + w]
                conv(w, 1)
                yb = y_s[:, :w].astype(bf16)
                ud = (u_s[:, c0:c0 + w].astype(f32) * dsk_ref[:, c0:c0 + w].astype(f32)).astype(bf16)
                a_out = (yb.astype(f32) + ud.astype(f32)).astype(bf16)
                h_s[:, c0:c0 + w] = (x_ref[:, c0:c0 + w].astype(f32) + a_out.astype(f32)).astype(bf16)

            return
        kt_s = dk_s
        ddsk_ref[...] = jnp.sum(dh_s[...].astype(f32) * u_s[...].astype(f32), axis=0, keepdims=True).astype(bf16)
        for (c0, w) in LANES:
            build_sh(dh_s, c0, w, -1)
            dk_s[:, :w] = kt_full[:, c0:c0 + w]
            conv(w, -1)
            du = (y_s[:, :w].astype(bf16).astype(f32)
                  + (dh_s[:, c0:c0 + w].astype(f32) * dsk_ref[:, c0:c0 + w].astype(f32)).astype(bf16).astype(f32))
            h_s[:, c0:c0 + w] = du.astype(bf16)
            build_sh(u_s, c0, w, 1)
            y_s[:, :w] = dh_s[:, c0:c0 + w].astype(f32)
            for (rb, lb, ps, npp, terms) in CREG + [(641, 1016, 8, 1, [(4, 0), (5, 0)])]:
                ni = len(terms)

                def pbody(p, c, rb=rb, lb=lb, ps=ps, terms=terms, ni=ni):
                    v0 = lb + ps * p
                    i0 = jnp.maximum(v0 - 8, 0) // RB

                    def rbody(i, accs):
                        t0 = i * RB
                        dy = y_s[pl.ds(pl.multiple_of(t0, 8), RB), :w]
                        new = []
                        for j, (a, eo) in enumerate(terms):
                            st = PAD + t0 - (v0 + eo)
                            pr = dy * sh_s[a, pl.ds(pl.multiple_of(st, 8), RB), :w]
                            new.append(accs[j] + jnp.sum(pr.reshape(RB // 8, 8, w), axis=0))
                        return tuple(new)
                    accs = lax.fori_loop(i0, L // RB, rbody, tuple(jnp.zeros((8, w), f32) for _ in terms))
                    for j in range(ni):
                        dk_s[pl.ds(rb + ni * p + j, 1), :w] = jnp.sum(accs[j], axis=0, keepdims=True)
                    return c
                lax.fori_loop(0, npp, pbody, 0)
            dk_s[256:257, :w] = dk_s[256:257, :w] - dk_s[255:256, :w]
            dk_s[384:385, :w] = dk_s[384:385, :w] - dk_s[383:384, :w]
            dk_s[512:513, :w] = dk_s[512:513, :w] - dk_s[641:642, :w] - dk_s[642:643, :w]
            dt, A_r, A_i, B_r, B_i, C_r, C_i, ar, ai, dbr, dbi, wr, wi = ssm_params(c0, w)
            build_lo(ar, ai, w)
            er, ei = cexp(ar, ai, 2048.0)
            k = dk_s[640:641, :w]
            G = (k * er, k * ei, 2048.0 * k * er, 2048.0 * k * ei)
            for g, (rb, lb, s, nh) in enumerate(REG):
                def gbody(a, G, g=g, rb=rb, lb=lb, s=s):
                    l0 = (lb + 16 * s * a).astype(f32)
                    er, ei = cexp(ar, ai, l0)
                    kk = dk_s[pl.ds(pl.multiple_of(rb + 16 * a, 8), 16), :w]
                    z = jnp.zeros((N, w), f32)
                    i0r, i0i, i1r, i1i = z, z, z, z
                    for b in range(16):
                        k = kk[b:b + 1, :]
                        lr, li = lo_s[g, b, 0, :, :w], lo_s[g, b, 1, :, :w]
                        i0r, i0i = i0r + k * lr, i0i + k * li
                        kb = k * float(s * b)
                        i1r, i1i = i1r + kb * lr, i1i + kb * li
                    i1r, i1i = i1r + l0 * i0r, i1i + l0 * i0i
                    return (G[0] + er * i0r - ei * i0i, G[1] + er * i0i + ei * i0r,
                            G[2] + er * i1r - ei * i1i, G[3] + er * i1i + ei * i1r)
                G = lax.fori_loop(0, nh, gbody, G)
            dwr, dwi = G[0], -G[1]
            sl = slice(c0, c0 + w)
            dcre_ref[:, sl] = (dwr * dbr + dwi * dbi).astype(bf16)
            dcim_ref[:, sl] = (-dwr * dbi + dwi * dbr).astype(bf16)
            ddbr, ddbi = dwr * C_r + dwi * C_i, -dwr * C_i + dwi * C_r
            dbre_ref[:, sl] = (dt * ddbr).astype(bf16)
            dbim_ref[:, sl] = (dt * ddbi).astype(bf16)
            dar, dai = wr * G[2] - wi * G[3], -(wr * G[3] + wi * G[2])
            dare_ref[:, sl] = (dt * dar).astype(bf16)
            daim_ref[:, sl] = (dt * dai).astype(bf16)
            ddt = jnp.sum(ddbr * B_r + ddbi * B_i + dar * A_r + dai * A_i, axis=0, keepdims=True)
            dldt_ref[:, sl] = (ddt * dt).astype(bf16)

    def blockb(tr_s, zb_s, z2_s, g_s, acc_s):
        def f1(i, c):
            xh, _ = _ln(h_s[rows(i), :].astype(f32))
            x2 = xh.astype(bf16)
            x2_s[rows(i), :] = x2
            for j in range(4):
                cs = slice(j * 1152, (j + 1) * 1152)
                zb_s[rows(i), cs] = _dot(x2, win_ref[:, cs]).astype(bf16)
            z = _gelu(zb_s[rows(i), FH:].astype(f32)).astype(bf16).astype(f32)
            zh, _ = _ln(z)
            z2_s[rows(i), :] = zh.astype(bf16)
            return c
        lax.fori_loop(0, nblk, f1, 0)

        tr_s[...] = go_ref[...].astype(f32).T.astype(bf16)
        acc_s[...] = jnp.zeros(acc_s.shape, f32)

        def f2(i, c):
            go = go_ref[rows(i), :]
            gs = []
            for j in range(2):
                cs = slice(j * 1152, (j + 1) * 1152)
                gs.append((_dot(wsp_ref[rows(i), :], z2_s[:, cs]).astype(bf16).astype(f32)
                           + bsp_ref[rows(i), :].astype(f32)).astype(bf16).astype(f32))
            g = jnp.concatenate(gs, axis=1)
            zp = zb_s[rows(i), :FH].astype(f32)
            z1 = _gelu(zp).astype(bf16).astype(f32)
            a1 = (z1 * g).astype(bf16)
            o = _dot(a1, wout_ref[...]).astype(bf16).astype(f32)
            out_ref[rows(i), :] = (h_s[rows(i), :].astype(f32) + o).astype(bf16)
            acc_s[...] += _dot(tr_s[:, rows(i)], a1)
            da1 = _dot_nt(go, wout_ref[...]).astype(bf16).astype(f32)
            dg = (da1 * z1).astype(bf16)
            g_s[rows(i), :] = dg
            dbsp_ref[rows(i), :] = jnp.sum(dg.astype(f32), axis=1, keepdims=True).astype(bf16)
            dz1 = (da1 * g).astype(bf16).astype(f32)
            zb_s[rows(i), :FH] = (dz1 * _gelu_grad(zp)).astype(bf16)
            return c
        lax.fori_loop(0, nblk, f2, 0)
        dwoutt_ref[...] = acc_s[...].astype(bf16)

        def b1(i, c):
            dgi = g_s[rows(i), :]
            for j in range(4):
                cs = pl.ds(j * 512, 512)
                dwsp_ref[rows(i), cs] = _dot_nt(dgi, z2_s[cs, :]).astype(bf16)
            ds = []
            for j in range(2):
                cs = slice(j * 1152, (j + 1) * 1152)
                ds.append(_dot(wspt_ref[rows(i), :], g_s[:, cs]).astype(bf16).astype(f32))
            dz2 = jnp.concatenate(ds, axis=1)
            zp = zb_s[rows(i), FH:].astype(f32)
            z = _gelu(zp).astype(bf16).astype(f32)
            zh, r = _ln(z)
            dz = _ln_bwd(zh, r, dz2).astype(bf16).astype(f32)
            zb_s[rows(i), FH:] = (dz * _gelu_grad(zp)).astype(bf16)
            return c
        lax.fori_loop(0, nblk, b1, 0)

        tr_s[...] = x2_s[...].astype(f32).T.astype(bf16)
        for j in range(6):
            cs = slice(j * 768, (j + 1) * 768)
            dwin_ref[:, cs] = _dot(tr_s[...], zb_s[:, cs]).astype(bf16)

        def b2(i, c):
            dx2 = _dot_nt(zb_s[rows(i), :], win_ref[...]).astype(bf16).astype(f32)
            xh, r = _ln(h_s[rows(i), :].astype(f32))
            dh = (go_ref[rows(i), :].astype(f32) + _ln_bwd(xh, r, dx2).astype(bf16).astype(f32)).astype(bf16)
            x2_s[rows(i), :] = dh
            return c
        lax.fori_loop(0, nblk, b2, 0)

    pl.run_scoped(functools.partial(ssm, True),
        pltpu.VMEM((13, L + 2 * PAD, 128), f32), pltpu.VMEM((L + 2 * PAD + 16, 128), f32),
        pltpu.VMEM((4, 16, 2, N, 128), f32), pltpu.VMEM((NQ, 128), f32), pltpu.VMEM((L, 128), f32))
    pl.run_scoped(blockb, pltpu.VMEM((D, L), bf16), pltpu.VMEM((L, 2 * FH), bf16), pltpu.VMEM((L, FH), bf16),
        pltpu.VMEM((L, FH), bf16), pltpu.VMEM((D, FH), f32))
    pl.run_scoped(functools.partial(ssm, False),
        pltpu.VMEM((13, L + 2 * PAD, 128), f32), pltpu.VMEM((L + 2 * PAD + 16, 128), f32),
        pltpu.VMEM((4, 16, 2, N, 128), f32), pltpu.VMEM((NQ, 128), f32), pltpu.VMEM((L, 128), f32))

    def b3(i, c):
        xh, r = _ln(x_ref[rows(i), :].astype(f32))
        d = _ln_bwd(xh, r, h_s[rows(i), :].astype(f32)).astype(bf16).astype(f32)
        dx_ref[rows(i), :] = (dh_s[rows(i), :].astype(f32) + d).astype(bf16)
        return c
    lax.fori_loop(0, nblk, b3, 0)


@jax.jit
def pallas_sequential_preLN__ssm_conv_s4__mixer_gmlp__prompt_kernel(
    A_u, A_A_re, A_A_im, A_B_re, A_B_im, A_C_re, A_C_im, A_log_dt, A_Dskip,
    B_x, B_w_in, B_w_sp, B_b_sp, B_w_out, grad_out,
):
    S = jax.ShapeDtypeStruct
    out_shape = (
        S((L, D), bf16), S((L, D), bf16),
        *[S((N, D), bf16)] * 6, S((1, D), bf16), S((1, D), bf16),
        S((D, 2 * FH), bf16), S((L, L), bf16), S((L, 1), bf16), S((D, FH), bf16),
    )
    scratch = [pltpu.VMEM((L, D), bf16), pltpu.VMEM((L, D), bf16), pltpu.VMEM((L, D), bf16),
               pltpu.VMEM((NQ, D), f32)]
    r = pl.pallas_call(
        _kernel, out_shape=out_shape, scratch_shapes=scratch,
        compiler_params=pltpu.CompilerParams(vmem_limit_bytes=124 * 1024 * 1024),
    )(A_u[0], A_A_re.T, A_A_im.T, A_B_re.T, A_B_im.T, A_C_re.T, A_C_im.T,
      A_log_dt[None, :], A_Dskip[None, :], B_w_in, B_w_sp, B_w_sp.T, B_b_sp[:, None], B_w_out,
      grad_out[0])
    (o, dx, dar, dai, dbr, dbi, dcr, dci, dldt, ddsk, dwin, dwsp, dbsp, dwot) = r
    return (o[None], dx[None], dar.T, dai.T, dbr.T, dbi.T, dcr.T, dci.T, dldt[0], ddsk[0],
            dwin, dwsp, dbsp[:, 0], dwot.T)
```

```python
import functools
import jax
import jax.numpy as jnp
from jax import lax
import jax.experimental.pallas as pl
import jax.experimental.pallas.tpu as pltpu

L, D, N, FH = 2048, 576, 128, 2304
PAD = 160
RB = 128
TM = 256
NQ = 648
LANES = [(0, 128), (128, 128), (256, 128), (384, 128), (512, 64)]
REG = [(0, 0, 1, 16), (256, 256, 2, 8), (384, 512, 4, 8), (512, 1024, 8, 8)]
CREG = [
    (0, 0, 8, 32, [(r, 0) for r in range(8)]),
    (256, 256, 8, 32, [(8, 0), (2, 0), (9, 0), (6, 0)]),
    (384, 512, 8, 64, [(10, 0), (9, 0)]),
    (512, 1024, 16, 65, [(12, 0), (11, 8)]),
]
f32, bf16 = jnp.float32, jnp.bfloat16
_C0 = 0.7978845608028654


def _ln(x):
    m = jnp.mean(x, axis=-1, keepdims=True)
    c = x - m
    v = jnp.mean(c * c, axis=-1, keepdims=True)
    r = lax.rsqrt(v + 1e-5)
    return c * r, r


def _ln_bwd(xh, r, dy):
    a = jnp.mean(dy, axis=-1, keepdims=True)
    b = jnp.mean(dy * xh, axis=-1, keepdims=True)
    return r * (dy - a - xh * b)


def _gelu(x):
    return 0.5 * x * (1.0 + jnp.tanh(_C0 * (x + 0.044715 * x * x * x)))


def _gelu_grad(x):
    t = jnp.tanh(_C0 * (x + 0.044715 * x * x * x))
    return 0.5 * (1.0 + t) + 0.5 * x * (1.0 - t * t) * _C0 * (1.0 + 0.134145 * x * x)


def _dot(a, b):
    return jnp.dot(a, b, preferred_element_type=f32)


def _dot_nt(a, b):
    return lax.dot_general(a, b, (((1,), (1,)), ((), ())), preferred_element_type=f32)


def _kernel(x_ref, are_ref, aim_ref, bre_ref, bim_ref, cre_ref, cim_ref, ldt_ref, dsk_ref,
            win_ref, wsp_ref, wspt_ref, bsp_ref, wout_ref, go_ref,
            out_ref, dx_ref, dare_ref, daim_ref, dbre_ref, dbim_ref, dcre_ref, dcim_ref,
            dldt_ref, ddsk_ref, dwin_ref, dwsp_ref, dbsp_ref, dwoutt_ref,
            u_s, h_s, x2_s, kt_s):
    nblk = L // TM

    def rows(i):
        return pl.ds(pl.multiple_of(i * TM, TM), TM)

    def ln1(i, c):
        xh, _ = _ln(x_ref[rows(i), :].astype(f32))
        u_s[rows(i), :] = xh.astype(bf16)
        return c
    lax.fori_loop(0, nblk, ln1, 0)

    kt_full = kt_s
    dh_s = x2_s
    def ssm(fwd_pass, sh_s, up_s, lo_s, dk_s, y_s):
        kt_s = kt_full
        def ssm_params(c0, w):
            sl = slice(c0, c0 + w)
            dt = jnp.exp(ldt_ref[:, sl].astype(f32)).astype(bf16).astype(f32)
            A_r, A_i = are_ref[:, sl].astype(f32), aim_ref[:, sl].astype(f32)
            B_r, B_i = bre_ref[:, sl].astype(f32), bim_ref[:, sl].astype(f32)
            C_r, C_i = cre_ref[:, sl].astype(f32), cim_ref[:, sl].astype(f32)
            ar, ai = dt * A_r, dt * A_i
            dbr, dbi = dt * B_r, dt * B_i
            wr, wi = C_r * dbr - C_i * dbi, C_r * dbi + C_i * dbr
            return dt, A_r, A_i, B_r, B_i, C_r, C_i, ar, ai, dbr, dbi, wr, wi

        def cexp(ar, ai, l):
            e = jnp.exp(ar * l)
            return e * jnp.cos(ai * l), e * jnp.sin(ai * l)

        def build_lo(ar, ai, w):
            for g, (_, _, s, _) in enumerate(REG):
                e1r, e1i = cexp(ar, ai, float(s))
                er, ei = jnp.ones_like(e1r), jnp.zeros_like(e1r)
                for b in range(16):
                    lo_s[g, b, 0, :, :w] = er
                    lo_s[g, b, 1, :, :w] = ei
                    er, ei = er * e1r - ei * e1i, er * e1i + ei * e1r

        def build_sh(src, c0, w, sign):
            o = 8 + PAD
            up_s[...] = jnp.zeros(up_s.shape, f32)
            up_s[o:o + L, :w] = src[:, c0:c0 + w].astype(f32)
            R = L + 2 * PAD

            def sh(k):
                return up_s[8 - sign * k:8 - sign * k + R, :w]
            for r in range(8):
                sh_s[r, :, :w] = sh(r)
            s3 = sh(-1) + sh(0) + sh(1)
            sh_s[8, :, :w] = s3
            sh_s[9, :, :w] = sh(3) + sh(4) + sh(5)
            s5 = s3 + sh(-2) + sh(2)
            sh_s[10, :, :w] = s5
            s7 = s5 + sh(-3) + sh(3)
            sh_s[11, :, :w] = s7
            sh_s[12, :, :w] = s7 + sh(-4) + sh(4)

        def conv(w, sign):
            def blk(i, c):
                t0 = i * RB
                span = (t0 + RB) if sign > 0 else (L - t0)
                acc = jnp.zeros((RB, w), f32)
                for (rb, lb, ps, npp, terms) in CREG:
                    ni = len(terms)

                    def body(p, acc, rb=rb, lb=lb, ps=ps, terms=terms, ni=ni):
                        for j, (a, eo) in enumerate(terms):
                            k = kt_s[pl.ds(rb + ni * p + j, 1), :w]
                            st = PAD + t0 - sign * (lb + ps * p + eo)
                            acc = acc + k * sh_s[a, pl.ds(pl.multiple_of(st, 8), RB), :w]
                        return acc
                    hi = jnp.clip((span + 8 - lb) // ps + 1, 0, npp)
                    acc = lax.fori_loop(0, hi, body, acc)
                @pl.when(span > 1016)
                def _():
                    k = kt_s[pl.ds(641, 1), :w]
                    st = PAD + t0 - sign * 1016
                    e = sh_s[4, pl.ds(pl.multiple_of(st, 8), RB), :w] + sh_s[5, pl.ds(pl.multiple_of(st, 8), RB), :w]
                    y_s[pl.ds(pl.multiple_of(t0, 8), RB), :w] = acc + k * e

                @pl.when(span <= 1016)
                def _():
                    y_s[pl.ds(pl.multiple_of(t0, 8), RB), :w] = acc
                return c
            lax.fori_loop(0, L // RB, blk, 0)

        if fwd_pass:
            for (c0, w) in LANES:
                dt, A_r, A_i, B_r, B_i, C_r, C_i, ar, ai, dbr, dbi, wr, wi = ssm_params(c0, w)
                build_lo(ar, ai, w)
                for g, (rb, lb, s, nh) in enumerate(REG):
                    def kbody(a, c, g=g, rb=rb, lb=lb, s=s):
                        er, ei = cexp(ar, ai, (lb + 16 * s * a).astype(f32))
                        hr, hi = wr * er - wi * ei, wr * ei + wi * er
                        for half in range(2):
                            rws = [jnp.sum(hr * lo_s[g, b, 0, :, :w] - hi * lo_s[g, b, 1, :, :w], axis=0, keepdims=True)
                                   for b in range(8 * half, 8 * half + 8)]
                            kt_s[pl.ds(pl.multiple_of(rb + 16 * a + 8 * half, 8), 8), c0:c0 + w] = jnp.concatenate(rws, axis=0)
                        return c
                    lax.fori_loop(0, nh, kbody, 0)
                er, ei = cexp(ar, ai, 2048.0)
                k2048 = jnp.sum(wr * er - wi * ei, axis=0, keepdims=True)
                k1024 = kt_s[512:513, c0:c0 + w]
                kt_s[640:648, c0:c0 + w] = jnp.concatenate(
                    [k2048, -k1024] + [jnp.zeros_like(k2048)] * 6, axis=0)
                kt_s[255:256, c0:c0 + w] = kt_s[255:256, c0:c0 + w] - kt_s[256:257, c0:c0 + w]
                kt_s[383:384, c0:c0 + w] = kt_s[383:384, c0:c0 + w] - kt_s[384:385, c0:c0 + w]

            for (c0, w) in LANES:
                build_sh(u_s, c0, w, 1)
                kt_s = kt_full.at[:, c0:c0 + w] if False else kt_full
                kt_s = dk_s
                dk_s[:, :w] = kt_full[:, c0:c0 + w]
                conv(w, 1)
                yb = y_s[:, :w].astype(bf16)
                ud = (u_s[:, c0:c0 + w].astype(f32) * dsk_ref[:, c0:c0 + w].astype(f32)).astype(bf16)
                a_out = (yb.astype(f32) + ud.astype(f32)).astype(bf16)
                h_s[:, c0:c0 + w] = (x_ref[:, c0:c0 + w].astype(f32) + a_out.astype(f32)).astype(bf16)

            return
        kt_s = dk_s
        ddsk_ref[...] = jnp.sum(dh_s[...].astype(f32) * u_s[...].astype(f32), axis=0, keepdims=True).astype(bf16)
        for (c0, w) in LANES:
            build_sh(dh_s, c0, w, -1)
            dk_s[:, :w] = kt_full[:, c0:c0 + w]
            conv(w, -1)
            du = (y_s[:, :w].astype(bf16).astype(f32)
                  + (dh_s[:, c0:c0 + w].astype(f32) * dsk_ref[:, c0:c0 + w].astype(f32)).astype(bf16).astype(f32))
            h_s[:, c0:c0 + w] = du.astype(bf16)
            build_sh(u_s, c0, w, 1)
            y_s[:, :w] = dh_s[:, c0:c0 + w].astype(f32)
            for (rb, lb, ps, npp, terms) in CREG + [(641, 1016, 8, 1, [(4, 0), (5, 0)])]:
                ni = len(terms)

                def pbody(p, c, rb=rb, lb=lb, ps=ps, terms=terms, ni=ni):
                    v0 = lb + ps * p
                    i0 = jnp.maximum(v0 - 8, 0) // RB

                    def rbody(i, accs):
                        t0 = i * RB
                        dy = y_s[pl.ds(pl.multiple_of(t0, 8), RB), :w]
                        new = []
                        for j, (a, eo) in enumerate(terms):
                            st = PAD + t0 - (v0 + eo)
                            pr = dy * sh_s[a, pl.ds(pl.multiple_of(st, 8), RB), :w]
                            new.append(accs[j] + jnp.sum(pr.reshape(RB // 8, 8, w), axis=0))
                        return tuple(new)
                    accs = lax.fori_loop(i0, L // RB, rbody, tuple(jnp.zeros((8, w), f32) for _ in terms))
                    for j in range(ni):
                        dk_s[pl.ds(rb + ni * p + j, 1), :w] = jnp.sum(accs[j], axis=0, keepdims=True)
                    return c
                lax.fori_loop(0, npp, pbody, 0)
            dk_s[256:257, :w] = dk_s[256:257, :w] - dk_s[255:256, :w]
            dk_s[384:385, :w] = dk_s[384:385, :w] - dk_s[383:384, :w]
            dk_s[512:513, :w] = dk_s[512:513, :w] - dk_s[641:642, :w] - dk_s[642:643, :w]
            dt, A_r, A_i, B_r, B_i, C_r, C_i, ar, ai, dbr, dbi, wr, wi = ssm_params(c0, w)
            build_lo(ar, ai, w)
            er, ei = cexp(ar, ai, 2048.0)
            k = dk_s[640:641, :w]
            G = (k * er, k * ei, 2048.0 * k * er, 2048.0 * k * ei)
            for g, (rb, lb, s, nh) in enumerate(REG):
                def gbody(a, G, g=g, rb=rb, lb=lb, s=s):
                    l0 = (lb + 16 * s * a).astype(f32)
                    er, ei = G[4], G[5]
                    kk = dk_s[pl.ds(pl.multiple_of(rb + 16 * a, 8), 16), :w]
                    parts = []
                    for n0 in range(0, N, 32):
                        z = jnp.zeros((32, w), f32)
                        i0r, i0i, i1r, i1i = z, z, z, z
                        for b in range(16):
                            k = kk[b:b + 1, :]
                            lr, li = lo_s[g, b, 0, n0:n0 + 32, :w], lo_s[g, b, 1, n0:n0 + 32, :w]
                            i0r, i0i = i0r + k * lr, i0i + k * li
                            kb = k * float(s * b)
                            i1r, i1i = i1r + kb * lr, i1i + kb * li
                        parts.append((i0r, i0i, i1r, i1i))
                    i0r, i0i, i1r, i1i = [jnp.concatenate([q[m] for q in parts], axis=0) for m in range(4)]
                    i1r, i1i = i1r + l0 * i0r, i1i + l0 * i0i
                    return (G[0] + er * i0r - ei * i0i, G[1] + er * i0i + ei * i0r,
                            G[2] + er * i1r - ei * i1i, G[3] + er * i1i + ei * i1r,
                        er * sr - ei * si, er * si + ei * sr)
                sr, si = cexp(ar, ai, float(16 * s))
                G = tuple(G[:4]) + cexp(ar, ai, float(lb))
                G = lax.fori_loop(0, nh, gbody, G)
            dwr, dwi = G[0], -G[1]
            sl = slice(c0, c0 + w)
            dcre_ref[:, sl] = (dwr * dbr + dwi * dbi).astype(bf16)
            dcim_ref[:, sl] = (-dwr * dbi + dwi * dbr).astype(bf16)
            ddbr, ddbi = dwr * C_r + dwi * C_i, -dwr * C_i + dwi * C_r
            dbre_ref[:, sl] = (dt * ddbr).astype(bf16)
            dbim_ref[:, sl] = (dt * ddbi).astype(bf16)
            dar, dai = wr * G[2] - wi * G[3], -(wr * G[3] + wi * G[2])
            dare_ref[:, sl] = (dt * dar).astype(bf16)
            daim_ref[:, sl] = (dt * dai).astype(bf16)
            ddt = jnp.sum(ddbr * B_r + ddbi * B_i + dar * A_r + dai * A_i, axis=0, keepdims=True)
            dldt_ref[:, sl] = (ddt * dt).astype(bf16)

    def blockb(tr_s, zb_s, z2_s, g_s, acc_s):
        def f1(i, c):
            xh, _ = _ln(h_s[rows(i), :].astype(f32))
            x2 = xh.astype(bf16)
            x2_s[rows(i), :] = x2
            for j in range(4):
                cs = slice(j * 1152, (j + 1) * 1152)
                zb_s[rows(i), cs] = _dot(x2, win_ref[:, cs]).astype(bf16)
            z = _gelu(zb_s[rows(i), FH:].astype(f32)).astype(bf16).astype(f32)
            zh, _ = _ln(z)
            z2_s[rows(i), :] = zh.astype(bf16)
            return c
        lax.fori_loop(0, nblk, f1, 0)

        tr_s[...] = go_ref[...].astype(f32).T.astype(bf16)
        acc_s[...] = jnp.zeros(acc_s.shape, f32)

        def f2(i, c):
            go = go_ref[rows(i), :]
            gs = []
            for j in range(2):
                cs = slice(j * 1152, (j + 1) * 1152)
                gs.append((_dot(wsp_ref[rows(i), :], z2_s[:, cs]).astype(bf16).astype(f32)
                           + bsp_ref[rows(i), :].astype(f32)).astype(bf16).astype(f32))
            g = jnp.concatenate(gs, axis=1)
            zp = zb_s[rows(i), :FH].astype(f32)
            z1 = _gelu(zp).astype(bf16).astype(f32)
            a1 = (z1 * g).astype(bf16)
            o = _dot(a1, wout_ref[...]).astype(bf16).astype(f32)
            out_ref[rows(i), :] = (h_s[rows(i), :].astype(f32) + o).astype(bf16)
            acc_s[...] += _dot(tr_s[:, rows(i)], a1)
            da1 = _dot_nt(go, wout_ref[...]).astype(bf16).astype(f32)
            dg = (da1 * z1).astype(bf16)
            g_s[rows(i), :] = dg
            dbsp_ref[rows(i), :] = jnp.sum(dg.astype(f32), axis=1, keepdims=True).astype(bf16)
            dz1 = (da1 * g).astype(bf16).astype(f32)
            zb_s[rows(i), :FH] = (dz1 * _gelu_grad(zp)).astype(bf16)
            return c
        lax.fori_loop(0, nblk, f2, 0)
        dwoutt_ref[...] = acc_s[...].astype(bf16)

        def b1(i, c):
            dgi = g_s[rows(i), :]
            for j in range(4):
                cs = pl.ds(j * 512, 512)
                dwsp_ref[rows(i), cs] = _dot_nt(dgi, z2_s[cs, :]).astype(bf16)
            ds = []
            for j in range(2):
                cs = slice(j * 1152, (j + 1) * 1152)
                ds.append(_dot(wspt_ref[rows(i), :], g_s[:, cs]).astype(bf16).astype(f32))
            dz2 = jnp.concatenate(ds, axis=1)
            zp = zb_s[rows(i), FH:].astype(f32)
            z = _gelu(zp).astype(bf16).astype(f32)
            zh, r = _ln(z)
            dz = _ln_bwd(zh, r, dz2).astype(bf16).astype(f32)
            zb_s[rows(i), FH:] = (dz * _gelu_grad(zp)).astype(bf16)
            return c
        lax.fori_loop(0, nblk, b1, 0)

        tr_s[...] = x2_s[...].astype(f32).T.astype(bf16)
        for j in range(6):
            cs = slice(j * 768, (j + 1) * 768)
            dwin_ref[:, cs] = _dot(tr_s[...], zb_s[:, cs]).astype(bf16)

        def b2(i, c):
            dx2 = _dot_nt(zb_s[rows(i), :], win_ref[...]).astype(bf16).astype(f32)
            xh, r = _ln(h_s[rows(i), :].astype(f32))
            dh = (go_ref[rows(i), :].astype(f32) + _ln_bwd(xh, r, dx2).astype(bf16).astype(f32)).astype(bf16)
            x2_s[rows(i), :] = dh
            return c
        lax.fori_loop(0, nblk, b2, 0)

    pl.run_scoped(functools.partial(ssm, True),
        pltpu.VMEM((13, L + 2 * PAD, 128), f32), pltpu.VMEM((L + 2 * PAD + 16, 128), f32),
        pltpu.VMEM((4, 16, 2, N, 128), f32), pltpu.VMEM((NQ, 128), f32), pltpu.VMEM((L, 128), f32))
    pl.run_scoped(blockb, pltpu.VMEM((D, L), bf16), pltpu.VMEM((L, 2 * FH), bf16), pltpu.VMEM((L, FH), bf16),
        pltpu.VMEM((L, FH), bf16), pltpu.VMEM((D, FH), f32))
    pl.run_scoped(functools.partial(ssm, False),
        pltpu.VMEM((13, L + 2 * PAD, 128), f32), pltpu.VMEM((L + 2 * PAD + 16, 128), f32),
        pltpu.VMEM((4, 16, 2, N, 128), f32), pltpu.VMEM((NQ, 128), f32), pltpu.VMEM((L, 128), f32))

    def b3(i, c):
        xh, r = _ln(x_ref[rows(i), :].astype(f32))
        d = _ln_bwd(xh, r, h_s[rows(i), :].astype(f32)).astype(bf16).astype(f32)
        dx_ref[rows(i), :] = (dh_s[rows(i), :].astype(f32) + d).astype(bf16)
        return c
    lax.fori_loop(0, nblk, b3, 0)


@jax.jit
def pallas_sequential_preLN__ssm_conv_s4__mixer_gmlp__prompt_kernel(
    A_u, A_A_re, A_A_im, A_B_re, A_B_im, A_C_re, A_C_im, A_log_dt, A_Dskip,
    B_x, B_w_in, B_w_sp, B_b_sp, B_w_out, grad_out,
):
    S = jax.ShapeDtypeStruct
    out_shape = (
        S((L, D), bf16), S((L, D), bf16),
        *[S((N, D), bf16)] * 6, S((1, D), bf16), S((1, D), bf16),
        S((D, 2 * FH), bf16), S((L, L), bf16), S((L, 1), bf16), S((D, FH), bf16),
    )
    scratch = [pltpu.VMEM((L, D), bf16), pltpu.VMEM((L, D), bf16), pltpu.VMEM((L, D), bf16),
               pltpu.VMEM((NQ, D), f32)]
    r = pl.pallas_call(
        _kernel, out_shape=out_shape, scratch_shapes=scratch,
        compiler_params=pltpu.CompilerParams(vmem_limit_bytes=124 * 1024 * 1024),
    )(A_u[0], A_A_re.T, A_A_im.T, A_B_re.T, A_B_im.T, A_C_re.T, A_C_im.T,
      A_log_dt[None, :], A_Dskip[None, :], B_w_in, B_w_sp, B_w_sp.T, B_b_sp[:, None], B_w_out,
      grad_out[0])
    (o, dx, dar, dai, dbr, dbi, dcr, dci, dldt, ddsk, dwin, dwsp, dbsp, dwot) = r
    return (o[None], dx[None], dar.T, dai.T, dbr.T, dbi.T, dcr.T, dci.T, dldt[0], ddsk[0],
            dwin, dwsp, dbsp[:, 0], dwot.T)
```
